```python
import os as _os
_os.environ.setdefault("JAX_PLATFORMS", "cpu")
import jax
import jax.numpy as jnp

def _softmax(x, axis=-1):
    return jax.nn.softmax(x, axis=axis)
def _gelu(x):
    return jax.nn.gelu(x, approximate=True)
def _silu(x):
    return jax.nn.silu(x)
def _sigmoid(x):
    return jax.nn.sigmoid(x)
def _layernorm(x, axis=-1, eps=1e-5):
    m = jnp.mean(x, axis=axis, keepdims=True)
    v = jnp.var(x, axis=axis, keepdims=True)
    return (x - m) / jnp.sqrt(v + eps)
def _scatter_add(tgt, idx, src, axis=0):
    return tgt.at[idx].add(src)
def _segment_sum(src, seg, n):
    return jax.ops.segment_sum(src, seg, n)
class _Rng:
    def __init__(self, key):
        self._k = key
    def _next(self):
        self._k, sub = jax.random.split(self._k)
        return sub
    def normal(self, shape):
        return jax.random.normal(self._next(), shape, dtype=jnp.bfloat16)
    def randint(self, lo, hi, shape):
        return jax.random.randint(self._next(), shape, lo, hi, dtype=jnp.int32)
    def uniform(self, shape, lo=0.0, hi=1.0):
        return jax.random.uniform(self._next(), shape, jnp.bfloat16, lo, hi)
    def permutation(self, n):
        return jax.random.permutation(self._next(), n)


kernel_name = 'sequential_preLN__linear_kernel_hedgehog__dense_activation_squared_relu__prompt'

def setup_inputs():
    _rng = _Rng(jax.random.key(int.from_bytes(__import__("os").urandom(4), "little")))
    _w = (lambda a: (lambda t: t.astype(jnp.bfloat16) if jnp.issubdtype(t.dtype, jnp.floating) else t)(jnp.asarray(a)))
    def _A_setup():
        B, S, D, H = 1, 2048, 512, 32
        Dh = D // H
        return {
            "x": _w((lambda *s: _rng.normal(s) * 0.05)(B, S, D)),
            "wqkv": _w((lambda *s: _rng.normal(s) * 0.2)(D, 3 * D)),
            "w_phi": _w((lambda *s: _rng.normal(s) * 0.2)(H, Dh, Dh) * (Dh ** -0.5)),
            "wo": _w((lambda *s: _rng.normal(s) * 0.05)(D, D)),
        }
    _A_in = _A_setup()

    def _B_setup():
        B, S, D, F = 1, 2048, 512, 1792
        return {
            "x": _w((lambda *s: _rng.normal(s) * 0.05)(B, S, D)),
            "w1": _w((lambda *s: _rng.normal(s) * 0.05)(D, F)),
            "b1": _w((lambda *s: _rng.normal(s) * 0.05)(F)),
            "w2": _w((lambda *s: _rng.normal(s) * 0.05)(F, D)),
            "b2": _w((lambda *s: _rng.normal(s) * 0.05)(D)),
        }
    _B_in = _B_setup()

    return {
        "A_x": _A_in["x"],
        "A_wqkv": _A_in["wqkv"],
        "A_w_phi": _A_in["w_phi"],
        "A_wo": _A_in["wo"],
        "B_x": _B_in["x"],
        "B_w1": _B_in["w1"],
        "B_b1": _B_in["b1"],
        "B_w2": _B_in["w2"],
        "B_b2": _B_in["b2"],
    }

def reference(A_x, A_wqkv, A_w_phi, A_wo, B_x, B_w1, B_b1, B_w2, B_b2):
    def _A_ref(x, wqkv, w_phi, wo):
        B, S, D = x.shape
        H = 32; Dh = D // H
        qkv = (lambda x, *d: x.transpose(*d))((x @ wqkv).reshape(B, S, 3, H, Dh), 2, 0, 3, 1, 4)
        q, k, v = qkv[0], qkv[1], qkv[2]
        pq = jnp.einsum("bhsd,hdf->bhsf", q, w_phi)
        pk = jnp.einsum("bhsd,hdf->bhsf", k, w_phi)
        phi_q = jnp.concatenate([_softmax(pq, axis=-1), _softmax(-pq, axis=-1)], axis=-1)
        phi_k = jnp.concatenate([_softmax(pk, axis=-1), _softmax(-pk, axis=-1)], axis=-1)
        kv = jnp.einsum("bhsf,bhsd->bhfd", phi_k, v)
        z  = jnp.einsum("bhsf->bhf", phi_k)
        num = jnp.einsum("bhqf,bhfd->bhqd", phi_q, kv)
        den = jnp.einsum("bhqf,bhf->bhq", phi_q, z)[..., None] + 1e-6
        o = num / den
        return (lambda x, *d: x.transpose(*d))(o, 0, 2, 1, 3).reshape(B, S, D) @ wo

    def _B_ref(x, w1, b1, w2, b2):
        h = jnp.einsum("bsd,df->bsf", x, w1) + b1
        zero = jnp.zeros_like(h)
        r = jnp.where(h > zero, h, zero)
        h = r * r
        out = jnp.einsum("bsf,fd->bsd", h, w2) + b2
        return out

    x = A_x
    h = x + _A_ref(_layernorm(x, axis=-1), A_wqkv, A_w_phi, A_wo)
    h2 = h + _B_ref(_layernorm(h, axis=-1), B_w1, B_b1, B_w2, B_b2)
    return h2
```

```python
import functools

import jax
import jax.numpy as jnp
import jax.experimental.pallas as pl
import jax.experimental.pallas.tpu as pltpu

_LOG2E = 1.4426950408889634
_LN_EPS = 1e-5
_DEN_EPS = 1e-6
_H = 32
_G = 128
_TS = 512

_NT = (((1,), (1,)), ((), ()))
_NN = (((1,), (0,)), ((), ()))


def _dot(a, b, dims):
    return jax.lax.dot_general(a, b, dims, preferred_element_type=jnp.float32)


def _layernorm(x):
    m = jnp.mean(x, axis=-1, keepdims=True)
    xc = x - m
    v = jnp.mean(xc * xc, axis=-1, keepdims=True)
    return xc * jax.lax.rsqrt(v + _LN_EPS)


def _dual_softmax(p, ts):
    p3 = p.reshape(16, 8, ts)
    mx = jnp.max(p3, axis=0, keepdims=True)
    mn = jnp.min(p3, axis=0, keepdims=True)
    ep = jnp.exp2(p3 - mx)
    en = jnp.exp2(mn - p3)
    rp = 1.0 / jnp.sum(ep, axis=0, keepdims=True)
    rn = 1.0 / jnp.sum(en, axis=0, keepdims=True)
    return (ep * rp).reshape(128, ts), (en * rn).reshape(128, ts)


def _kernel(x_hbm, wqkv_hbm, wphi_hbm, wo_hbm, w1_hbm, b1_hbm, w2_hbm, b2_hbm,
            o_hbm,
            x_v, xn_v, wqkv_v, wphi_v, wo_v, w1_v, b1_v, w2_v, b2_v, o_v,
            wqT_v, wkT_v, wop_v, kv_acc, z_acc, a_v,
            x_sem, w_sem, o_sem, *, S, D, F):
    nt = S // _TS
    ng = D // _G
    bf16 = jnp.bfloat16

    def x_copy(i):
        return pltpu.make_async_copy(x_hbm.at[pl.ds(i * _TS, _TS)],
                                     x_v.at[pl.ds(i * _TS, _TS)], x_sem.at[i])

    def o_copy(i):
        return pltpu.make_async_copy(o_v.at[pl.ds(i * _TS, _TS)],
                                     o_hbm.at[pl.ds(i * _TS, _TS)], o_sem.at[i])

    c_wqkv = pltpu.make_async_copy(wqkv_hbm, wqkv_v, w_sem.at[0])
    c_wphi = pltpu.make_async_copy(wphi_hbm, wphi_v, w_sem.at[1])
    c_rest = [
        pltpu.make_async_copy(wo_hbm, wo_v, w_sem.at[2]),
        pltpu.make_async_copy(w1_hbm, w1_v, w_sem.at[3]),
        pltpu.make_async_copy(w2_hbm, w2_v, w_sem.at[4]),
        pltpu.make_async_copy(b1_hbm, b1_v, w_sem.at[5]),
        pltpu.make_async_copy(b2_hbm, b2_v, w_sem.at[6]),
    ]
    c_wphi.start()
    c_wqkv.start()
    for i in range(nt):
        x_copy(i).start()
    for c in c_rest:
        c.start()

    r128 = jax.lax.broadcasted_iota(jnp.int32, (_G, _G), 0)
    c128 = jax.lax.broadcasted_iota(jnp.int32, (_G, _G), 1)
    head_mask = (r128 % 8) == (c128 // 16)
    r16 = jax.lax.broadcasted_iota(jnp.int32, (_G, 16), 0)
    c16 = jax.lax.broadcasted_iota(jnp.int32, (_G, 16), 1)
    expand = jnp.where((r16 // 8) == c16, 1.0, 0.0).astype(bf16)
    perm = jnp.where(((r128 % 8) * 16 + r128 // 8) == c128, 1.0, 0.0).astype(bf16)

    c_wphi.wait()
    c_wqkv.wait()
    wphi = wphi_v[...].reshape(_H * 16, 16)
    for g in range(ng):
        t = _dot(expand, wphi[g * _G:(g + 1) * _G, :], _NT)
        t = jnp.where(head_mask, t, 0.0).astype(bf16)
        wq = _dot(t, wqkv_v[:, g * _G:(g + 1) * _G], _NT)
        wk = _dot(t, wqkv_v[:, D + g * _G:D + (g + 1) * _G], _NT)
        wqT_v[g * _G:(g + 1) * _G, :] = (wq * _LOG2E).astype(bf16)
        wkT_v[g * _G:(g + 1) * _G, :] = (wk * _LOG2E).astype(bf16)

    kv_acc[...] = jnp.zeros(kv_acc.shape, jnp.float32)
    z_acc[...] = jnp.zeros(z_acc.shape, jnp.float32)

    def phase1(i, carry):
        rows = pl.ds(pl.multiple_of(i * _TS, _TS), _TS)
        x_copy(i).wait()
        xn = _layernorm(x_v[rows, :].astype(jnp.float32)).astype(bf16)
        xn_v[rows, :] = xn
        pk = _dot(wkT_v[...], xn, _NT)
        v = _dot(xn, wqkv_v[:, 2 * D:3 * D], _NN).astype(bf16)
        for g in range(ng):
            fp, fn = _dual_softmax(pk[g * _G:(g + 1) * _G, :], _TS)
            phi = jnp.concatenate([fp, fn], axis=0)
            zs = phi[:, 0:128]
            for j in range(1, _TS // 128):
                zs = zs + phi[:, j * 128:(j + 1) * 128]
            z_acc[g] += zs
            kv_acc[g] += _dot(phi.astype(bf16), v[:, g * _G:(g + 1) * _G], _NN)
        return carry

    jax.lax.fori_loop(0, nt, phase1, 0)

    for c in c_rest:
        c.wait()
    r256 = jax.lax.broadcasted_iota(jnp.int32, (2 * _G, _G), 0)
    c256 = jax.lax.broadcasted_iota(jnp.int32, (2 * _G, _G), 1)
    kv_mask = (r256 % 8) == (c256 // 16)
    rz = jax.lax.broadcasted_iota(jnp.int32, (16, 2 * _G), 0)
    cz = jax.lax.broadcasted_iota(jnp.int32, (16, 2 * _G), 1)
    z_mask = rz == (cz % 8)
    ones = jnp.ones((16, _G), jnp.float32)
    for g in range(ng):
        kvm = jnp.where(kv_mask, kv_acc[g], 0.0).astype(bf16)
        a_v[g, 0:_G, :] = _dot(perm, kvm, _NT).astype(bf16)
        zrow = jax.lax.dot_general(ones, z_acc[g], _NT,
                                   precision=jax.lax.Precision.HIGHEST,
                                   preferred_element_type=jnp.float32)
        a_v[g, _G:_G + 16, :] = jnp.where(z_mask, zrow, 0.0).astype(bf16)
        wop_v[g * _G:(g + 1) * _G, :] = _dot(
            perm, wo_v[g * _G:(g + 1) * _G, :], _NN).astype(bf16)

    FC = 256

    def phase2(i, carry):
        rows = pl.ds(pl.multiple_of(i * _TS, _TS), _TS)
        xn = xn_v[rows, :]
        pq = _dot(wqT_v[...], xn, _NT)
        oT = []
        for g in range(ng):
            fp, fn = _dual_softmax(pq[g * _G:(g + 1) * _G, :], _TS)
            phi = jnp.concatenate([fp, fn], axis=0).astype(bf16)
            nd = _dot(a_v[g], phi, _NN)
            r = 1.0 / (nd[_G:_G + 8, :] + _DEN_EPS)
            oT.append((nd[0:_G, :].reshape(16, 8, _TS) * r[None]).reshape(_G, _TS))
        o = jnp.concatenate(oT, axis=0).T.astype(bf16)
        h = x_v[rows, :].astype(jnp.float32) + _dot(o, wop_v[...], _NN)
        hn = _layernorm(h).astype(bf16)
        acc = h + b2_v[...].astype(jnp.float32)
        for c in range(F // FC):
            cols = slice(c * FC, (c + 1) * FC)
            a = _dot(hn, w1_v[:, cols], _NN) + b1_v[:, cols].astype(jnp.float32)
            a = jnp.maximum(a, 0.0)
            acc = acc + _dot((a * a).astype(bf16), w2_v[cols, :], _NN)
        o_v[rows, :] = acc.astype(bf16)
        o_copy(i).start()
        return carry

    jax.lax.fori_loop(0, nt, phase2, 0)
    for i in range(nt):
        o_copy(i).wait()


@jax.jit
def pallas_sequential_preLN__linear_kernel_hedgehog__dense_activation_squared_relu__prompt_kernel(
    A_x: jax.Array,
    A_wqkv: jax.Array,
    A_w_phi: jax.Array,
    A_wo: jax.Array,
    B_x: jax.Array,
    B_w1: jax.Array,
    B_b1: jax.Array,
    B_w2: jax.Array,
    B_b2: jax.Array,
):
    del B_x
    B, S, D = A_x.shape
    F = B_w1.shape[1]
    assert B == 1 and D % _G == 0 and S % _TS == 0 and A_w_phi.shape == (_H, 16, 16)
    bf16, f32 = jnp.bfloat16, jnp.float32
    ng = D // _G
    nt = S // _TS
    any_spec = pl.BlockSpec(memory_space=pl.ANY)
    out = pl.pallas_call(
        functools.partial(_kernel, S=S, D=D, F=F),
        in_specs=[any_spec] * 8,
        out_specs=any_spec,
        out_shape=jax.ShapeDtypeStruct((S, D), A_x.dtype),
        scratch_shapes=[
            pltpu.VMEM((S, D), bf16),
            pltpu.VMEM((S, D), bf16),
            pltpu.VMEM((D, 3 * D), bf16),
            pltpu.VMEM((_H, 16, 16), bf16),
            pltpu.VMEM((D, D), bf16),
            pltpu.VMEM((D, F), bf16),
            pltpu.VMEM((1, F), bf16),
            pltpu.VMEM((F, D), bf16),
            pltpu.VMEM((1, D), bf16),
            pltpu.VMEM((S, D), bf16),
            pltpu.VMEM((D, D), bf16),
            pltpu.VMEM((D, D), bf16),
            pltpu.VMEM((D, D), bf16),
            pltpu.VMEM((ng, 2 * _G, _G), f32),
            pltpu.VMEM((ng, 2 * _G, _G), f32),
            pltpu.VMEM((ng, _G + 16, 2 * _G), bf16),
            pltpu.SemaphoreType.DMA((nt,)),
            pltpu.SemaphoreType.DMA((7,)),
            pltpu.SemaphoreType.DMA((nt,)),
        ],
        compiler_params=pltpu.CompilerParams(vmem_limit_bytes=100 * 1024 * 1024),
    )(A_x.reshape(S, D), A_wqkv, A_w_phi, A_wo, B_w1, B_b1.reshape(1, F), B_w2,
      B_b2.reshape(1, D))
    return out.reshape(B, S, D)
```

```python
import functools

import jax
import jax.numpy as jnp
import jax.experimental.pallas as pl
import jax.experimental.pallas.tpu as pltpu

_LOG2E = 1.4426950408889634
_LN_EPS = 1e-5
_DEN_EPS = 1e-6
_H = 32
_DH = 16
_G = 128
_TS = 512
_TAIL = 128
_FC = 256
_LN_ROWS = 128

_NT = (((1,), (1,)), ((), ()))
_NN = (((1,), (0,)), ((), ()))


def _dot(a, b, dims):
    return jax.lax.dot_general(a, b, dims, preferred_element_type=jnp.float32)


def _layernorm(x):
    out = []
    for r in range(0, x.shape[0], _LN_ROWS):
        xr = x[r:r + _LN_ROWS]
        xc = xr - jnp.mean(xr, axis=-1, keepdims=True)
        var = jnp.mean(xc * xc, axis=-1, keepdims=True)
        out.append((xc * jax.lax.rsqrt(var + _LN_EPS)).astype(jnp.bfloat16))
    return jnp.concatenate(out, axis=0)


def _dual_softmax(p):
    p3 = p.reshape(_DH, 8, p.shape[1])
    mx = jnp.max(p3, axis=0, keepdims=True)
    mn = jnp.min(p3, axis=0, keepdims=True)
    ep = jnp.exp2(p3 - mx)
    en = jnp.exp2(mn - p3)
    rp = 1.0 / jnp.sum(ep, axis=0, keepdims=True)
    rn = 1.0 / jnp.sum(en, axis=0, keepdims=True)
    return jnp.concatenate([ep * rp, en * rn], axis=0)


def _interleave(schedule, **gens):
    for name in schedule:
        next(gens[name])
    for gen in gens.values():
        for _ in gen:
            pass


def _kernel(x_hbm, wqkv_hbm, wphi_hbm, wo_hbm, w1_hbm, b1_hbm, w2_hbm, b2_hbm,
            o_hbm,
            x_v, xn_v, wqkv_v, wphi_v, wo_v, w1_v, b1_v, w2_v, b2_v, o_v,
            hn_v, h_v, t_v, wqT_v, wkT_v, kv_acc, z_acc, a_v, zb_v,
            x_sem, w_sem, o_sem, *, S, D, F):
    nt = S // _TS
    ng = D // _G
    bf16, f32 = jnp.bfloat16, jnp.float32

    def rows(i):
        if isinstance(i, int):
            return pl.ds(i * _TS, _TS)
        return pl.ds(pl.multiple_of(i * _TS, _TS), _TS)

    def x_copy(i):
        return pltpu.make_async_copy(x_hbm.at[rows(i)], x_v.at[rows(i)], x_sem.at[i])

    def o_copy(rr, sem):
        return pltpu.make_async_copy(o_v.at[rr], o_hbm.at[rr], o_sem.at[sem])

    def w_cols(j, sem):
        cols = slice(j * D, (j + 1) * D)
        return pltpu.make_async_copy(wqkv_hbm.at[:, cols], wqkv_v.at[:, cols], w_sem.at[sem])

    c_wq, c_wk, c_wv = w_cols(0, 0), w_cols(1, 1), w_cols(2, 2)
    c_wphi = pltpu.make_async_copy(wphi_hbm, wphi_v, w_sem.at[3])
    c_late = [
        c_wq,
        pltpu.make_async_copy(wo_hbm, wo_v, w_sem.at[4]),
        pltpu.make_async_copy(w1_hbm, w1_v, w_sem.at[5]),
        pltpu.make_async_copy(w2_hbm, w2_v, w_sem.at[6]),
        pltpu.make_async_copy(b1_hbm, b1_v, w_sem.at[7]),
        pltpu.make_async_copy(b2_hbm, b2_v, w_sem.at[8]),
    ]
    c_wphi.start()
    x_copy(0).start()
    c_wk.start()
    c_wv.start()

    kv_acc[...] = jnp.zeros(kv_acc.shape, f32)
    z_acc[...] = jnp.zeros(z_acc.shape, f32)

    r128 = jax.lax.broadcasted_iota(jnp.int32, (_G, _G), 0)
    c128 = jax.lax.broadcasted_iota(jnp.int32, (_G, _G), 1)
    head_mask = (r128 % 8) == (c128 // _DH)
    rg = jax.lax.broadcasted_iota(jnp.int32, (_G, _H), 0)
    cg = jax.lax.broadcasted_iota(jnp.int32, (_G, _H), 1)
    rf = jax.lax.broadcasted_iota(jnp.int32, (_G, 2 * _G), 0)
    cf = jax.lax.broadcasted_iota(jnp.int32, (_G, 2 * _G), 1)
    f_mask = (rf // 8) == (cf % _DH)
    rc = jax.lax.broadcasted_iota(jnp.int32, (2 * _G, _G), 0)
    cc = jax.lax.broadcasted_iota(jnp.int32, (2 * _G, _G), 1)
    gather_d = jnp.where((rc // _DH) == (cc % _DH), 1.0, 0.0).astype(bf16)
    kv_mask = (rc % 8) == (cc // _DH)

    c_wphi.wait()
    wphi = wphi_v[...].reshape(_DH * _DH, _H)
    for g in range(ng):
        pick = jnp.where(cg == (g * 8 + rg % 8), 1.0, 0.0).astype(bf16)
        y = jnp.where(f_mask, _dot(pick, wphi, _NT), 0.0).astype(bf16)
        t_v[g] = jnp.where(head_mask, _dot(y, gather_d, _NN), 0.0).astype(bf16)

    def fold(dst, col0):
        for g in range(ng):
            w = _dot(t_v[g], wqkv_v[:, col0 + g * _G:col0 + (g + 1) * _G], _NT)
            dst[g * _G:(g + 1) * _G, :] = (w * _LOG2E).astype(bf16)

    def ln1(i):
        xn_v[rows(i), :] = _layernorm(x_v[rows(i), :].astype(f32))

    x_copy(0).wait()
    c_wk.wait()
    ln1(0)
    fold(wkT_v, D)
    c_wv.wait()
    for i in range(1, nt):
        x_copy(i).start()

    for i in range(nt):
        if i == min(1, nt - 1):
            for c in c_late:
                c.start()
        xn = xn_v[rows(i), :]
        pk = _dot(wkT_v[...], xn, _NT)
        v = _dot(xn, wqkv_v[:, 2 * D:3 * D], _NN).astype(bf16)
        if 1 <= i < nt - 1:
            ln1(i + 1)
        phis = []
        for g in range(ng):
            phi = _dual_softmax(pk[g * _G:(g + 1) * _G, :]).reshape(2 * _G, _TS)
            z_acc[g] += (phi[:, 0:128] + phi[:, 128:256]) + (phi[:, 256:384] + phi[:, 384:512])
            phis.append(phi.astype(bf16))
        if i == 0:
            for j in range(1, nt):
                x_copy(j).wait()
            ln1(1)
        for g in range(ng):
            kv_acc[g] += _dot(phis[g], v[:, g * _G:(g + 1) * _G], _NN)

    for c in c_late:
        c.wait()

    def build_kv_operands():
        for g in range(ng):
            kvm = jnp.where(kv_mask, kv_acc[g], 0.0)
            a_v[g] = kvm.T.astype(bf16)
            z = jnp.sum(z_acc[g], axis=1, keepdims=True)
            zb_v[g] = jnp.broadcast_to(z, (2 * _G, _G))

    def attention(i, first=False):
        pq = _dot(wqT_v[...], xn_v[rows(i), :], _NT)
        yield
        if first:
            build_kv_operands()
        oT = []
        for g in range(ng):
            phi = _dual_softmax(pq[g * _G:(g + 1) * _G, :])
            zb = zb_v[g].reshape(2 * _DH, 8, _G)
            den = jnp.concatenate(
                [jnp.sum(phi[:, :, j * 128:(j + 1) * 128] * zb, axis=0)
                 for j in range(_TS // 128)], axis=1)
            r = 1.0 / (den + _DEN_EPS)
            num = _dot(a_v[g], phi.reshape(2 * _G, _TS).astype(bf16), _NN)
            for hl in range(8):
                oT.append(num[hl * _DH:(hl + 1) * _DH, :] * r[hl:hl + 1, :])
        o = jnp.concatenate(oT, axis=0).T.astype(bf16)
        yield
        h = x_v[rows(i), :].astype(f32) + _dot(o, wo_v[...], _NN)
        yield
        hn_v[rows(i), :] = _layernorm(h)
        h_v[rows(i), :] = h + b2_v[...].astype(f32).reshape(1, D)
        yield

    def ffn(rr, sem):
        b1 = b1_v[...].astype(f32).reshape(1, F)
        acc = None
        for c in range(F // _FC):
            cols = slice(c * _FC, (c + 1) * _FC)
            a = jnp.maximum(_dot(hn_v[rr, :], w1_v[:, cols], _NN) + b1[:, cols], 0.0)
            y = _dot((a * a).astype(bf16), w2_v[cols, :], _NN)
            acc = (h_v[rr, :] if acc is None else acc) + y
            yield
        o_v[rr, :] = acc.astype(bf16)
        o_copy(rr, sem).start()

    fold(wqT_v, 0)
    _interleave([], attn=attention(0, first=True))

    def phase2(i, carry):
        _interleave(["ffn", "attn"] * 4, attn=attention(i + 1), ffn=ffn(rows(i), i))
        return carry

    jax.lax.fori_loop(0, nt - 1, phase2, 0)

    last = (nt - 1) * _TS
    parts = [pl.ds(last, _TS - _TAIL), pl.ds(last + _TS - _TAIL, _TAIL)]
    for j in range(2):
        _interleave([], ffn=ffn(parts[j], nt - 1 + j))
    for i in range(nt - 1):
        o_copy(rows(i), i).wait()
    for j in range(2):
        o_copy(parts[j], nt - 1 + j).wait()


@jax.jit
def pallas_sequential_preLN__linear_kernel_hedgehog__dense_activation_squared_relu__prompt_kernel(
    A_x: jax.Array,
    A_wqkv: jax.Array,
    A_w_phi: jax.Array,
    A_wo: jax.Array,
    B_x: jax.Array,
    B_w1: jax.Array,
    B_b1: jax.Array,
    B_w2: jax.Array,
    B_b2: jax.Array,
):
    del B_x
    B, S, D = A_x.shape
    F = B_w1.shape[1]
    assert B == 1 and A_w_phi.shape == (_H, _DH, _DH) and D == _H * _DH
    assert _TS == 512 and S % _TS == 0 and S // _TS >= 2 and F % _FC == 0 and F // _FC >= 4
    bf16, f32 = jnp.bfloat16, jnp.float32
    ng = D // _G
    nt = S // _TS
    any_spec = pl.BlockSpec(memory_space=pl.ANY)
    out = pl.pallas_call(
        functools.partial(_kernel, S=S, D=D, F=F),
        in_specs=[any_spec] * 8,
        out_specs=any_spec,
        out_shape=jax.ShapeDtypeStruct((S, D), A_x.dtype),
        scratch_shapes=[
            pltpu.VMEM((S, D), bf16),
            pltpu.VMEM((S, D), bf16),
            pltpu.VMEM((D, 3 * D), bf16),
            pltpu.VMEM((_DH, _DH, _H), bf16),
            pltpu.VMEM((D, D), bf16),
            pltpu.VMEM((D, F), bf16),
            pltpu.VMEM((F,), bf16),
            pltpu.VMEM((F, D), bf16),
            pltpu.VMEM((D,), bf16),
            pltpu.VMEM((S, D), bf16),
            pltpu.VMEM((S, D), bf16),
            pltpu.VMEM((S, D), f32),
            pltpu.VMEM((ng, _G, _G), bf16),
            pltpu.VMEM((D, D), bf16),
            pltpu.VMEM((D, D), bf16),
            pltpu.VMEM((ng, 2 * _G, _G), f32),
            pltpu.VMEM((ng, 2 * _G, _G), f32),
            pltpu.VMEM((ng, _G, 2 * _G), bf16),
            pltpu.VMEM((ng, 2 * _G, _G), f32),
            pltpu.SemaphoreType.DMA((nt,)),
            pltpu.SemaphoreType.DMA((9,)),
            pltpu.SemaphoreType.DMA((nt + 1,)),
        ],
        compiler_params=pltpu.CompilerParams(vmem_limit_bytes=100 * 1024 * 1024),
    )(A_x.reshape(S, D), A_wqkv, A_w_phi.transpose(1, 2, 0), A_wo, B_w1, B_b1, B_w2,
      B_b2)
    return out.reshape(B, S, D)
```
